```python
import os as _os
_os.environ.setdefault('JAX_PLATFORMS', 'cpu')
import jax
import jax.numpy as jnp

def _softmax(x, axis=-1):
    return jax.nn.softmax(x, axis=axis)

def _gelu(x):
    return jax.nn.gelu(x, approximate=True)

def _silu(x):
    return jax.nn.silu(x)

def _sigmoid(x):
    return jax.nn.sigmoid(x)

def _layernorm(x, axis=-1, eps=1e-05):
    m = jnp.mean(x, axis=axis, keepdims=True)
    v = jnp.var(x, axis=axis, keepdims=True)
    return (x - m) / jnp.sqrt(v + eps)

def _scatter_add(tgt, idx, src, axis=0):
    return tgt.at[idx].add(src)

def _segment_sum(src, seg, n):
    return jax.ops.segment_sum(src, seg, n)

class _Rng:

    def __init__(self, key):
        self._k = key

    def _next(self):
        self._k, sub = jax.random.split(self._k)
        return sub

    def normal(self, shape):
        return jax.random.normal(self._next(), shape, dtype=jnp.bfloat16)

    def randint(self, lo, hi, shape):
        return jax.random.randint(self._next(), shape, lo, hi, dtype=jnp.int32)

    def uniform(self, shape, lo=0.0, hi=1.0):
        return jax.random.uniform(self._next(), shape, jnp.bfloat16, lo, hi)

    def permutation(self, n):
        return jax.random.permutation(self._next(), n)
kernel_name = 'gated_mix__memory_aug_recurrent_mem_tr__glu_gated_geglu__prompt'

def setup_inputs():
    _rng = _Rng(jax.random.key(int.from_bytes(__import__("os").urandom(4), "little")))
    _w = lambda a: (lambda t: t.astype(jnp.bfloat16) if jnp.issubdtype(t.dtype, jnp.floating) else t)(jnp.asarray(a))

    def _A_setup():
        B, S, Dm = (1, 2048, 640)
        H, Dh = (32, 128)
        M, seg = (8, 32)
        seg = min(seg, S)
        S = S // seg * seg
        return {'x': _w((lambda *s: _rng.normal(s) * 0.05)(B, S, Dm)), 'mem0': _w((lambda *s: _rng.normal(s) * 0.4)(B, M, Dm)), 'Wq': _w((lambda *s: _rng.normal(s) * 3.2)(Dm, H, Dh) * Dm ** (-0.5)), 'Wk': _w((lambda *s: _rng.normal(s) * 3.2)(Dm, H, Dh) * Dm ** (-0.5)), 'Wv': _w((lambda *s: _rng.normal(s) * 0.4)(Dm, H, Dh) * Dm ** (-0.5)), 'Wo': _w((lambda *s: _rng.normal(s) * 0.4)(H, Dh, Dm) * (H * Dh) ** (-0.5)), 'seg_len': seg}
    _A_in = _A_setup()

    def _B_setup():
        B, S, Dm, Df = (1, 2048, 640, 1728)
        return {'x': _w((lambda *s: _rng.normal(s) * 0.05)(B, S, Dm)), 'w_gate': _w((lambda *s: _rng.normal(s) * 1.6)(Dm, Df) * Dm ** (-0.5)), 'w_up': _w((lambda *s: _rng.normal(s) * 1.6)(Dm, Df) * Dm ** (-0.5)), 'w_down': _w((lambda *s: _rng.normal(s) * 1.6)(Df, Dm) * Df ** (-0.5))}
    _B_in = _B_setup()
    return {'A_x': _A_in['x'], 'A_mem0': _A_in['mem0'], 'A_Wq': _A_in['Wq'], 'A_Wk': _A_in['Wk'], 'A_Wv': _A_in['Wv'], 'A_Wo': _A_in['Wo'], 'A_seg_len': _A_in['seg_len'], 'B_x': _B_in['x'], 'B_w_gate': _B_in['w_gate'], 'B_w_up': _B_in['w_up'], 'B_w_down': _B_in['w_down'], 'gate_w': _w((lambda *s: _rng.normal(s) * 0.05)(640) * 16.0)}

def reference(A_x, A_mem0, A_Wq, A_Wk, A_Wv, A_Wo, A_seg_len, B_x, B_w_gate, B_w_up, B_w_down, gate_w):

    def _A_ref(x, mem0, Wq, Wk, Wv, Wo, seg_len):
        B, S, Dm = x.shape
        H, Dh = (Wq.shape[1], Wq.shape[2])
        M = mem0.shape[1]
        scale = Dh ** (-0.5)
        n_seg = S // seg_len
        L = M + seg_len
        idx = jnp.arange(L)
        mask = (idx[:, None] < M) | (idx[:, None] >= idx[None, :])
        mem = mem0
        outs = []
        for s in range(n_seg):
            xs = x[:, s * seg_len:(s + 1) * seg_len, :].copy()
            h = jnp.concatenate([mem, xs], axis=1)
            q = jnp.einsum('btd,dhe->bhte', h, Wq)
            k = jnp.einsum('btd,dhe->bhte', h, Wk)
            v = jnp.einsum('btd,dhe->bhte', h, Wv)
            scores = jnp.einsum('bhqe,bhke->bhqk', q, k) * scale
            scores = jnp.where(mask[None, None], scores, -1000000000.0)
            p = _softmax(scores, axis=-1)
            o = jnp.einsum('bhqk,bhke->bhqe', p, v)
            o = jnp.einsum('bhte,hed->btd', o, Wo)
            mem = o[:, :M, :].copy()
            outs.append(o[:, M:, :])
        return jnp.concatenate(outs, axis=1)

    def _B_ref(x, w_gate, w_up, w_down):
        g = jnp.einsum('bsd,df->bsf', x, w_gate)
        u = jnp.einsum('bsd,df->bsf', x, w_up)
        h = _gelu(g) * u
        return jnp.einsum('bsf,fd->bsd', h, w_down)
    x = A_x
    g = _sigmoid((x * gate_w).sum(-1, keepdims=True))
    a = _A_ref(x, A_mem0, A_Wq, A_Wk, A_Wv, A_Wo, A_seg_len)
    b = _B_ref(x, B_w_gate, B_w_up, B_w_down)
    return g * a + (1 - g) * b
```

```python
import functools
import jax
import jax.numpy as jnp
from jax import lax
import jax.experimental.pallas as pl
import jax.experimental.pallas.tpu as pltpu

BF = jnp.bfloat16
F32 = jnp.float32
U32 = jnp.uint32


def _dot(a, b):
    return jnp.dot(a, b, preferred_element_type=F32)


def _dot_nt(a, b):
    return lax.dot_general(a, b, (((1,), (1,)), ((), ())), preferred_element_type=F32)


def _bf(w32):
    return pltpu.bitcast(w32, BF)


def _cat0(*xs):
    return jnp.concatenate(xs, axis=0)


def _make_fill(order, L, M):
    r = lax.broadcasted_iota(jnp.int32, (2 * L, 2 * L), 0)
    c = lax.broadcasted_iota(jnp.int32, (2 * L, 2 * L), 1)
    rl = jnp.where(r >= L, r - L, r)
    cl = jnp.where(c >= L, c - L, c)
    same = ((r >= L) & (c >= L)) | ((r < L) & (c < L))

    def pos(l):
        p = l
        for (st, n, p0) in order:
            p = jnp.where((l >= st) & (l < st + n), l - st + p0, p)
        return p
    rp = pos(rl)
    cp = pos(cl)
    allowed = (rp < M) | (rp >= cp)
    fill = jnp.where(allowed, 0.0, -1e9).astype(F32)
    fill = jnp.where(same, fill, -3e38).astype(F32)
    return fill


@functools.partial(jax.jit, static_argnames=("A_seg_len",))
def pallas_gated_mix__memory_aug_recurrent_mem_tr__glu_gated_geglu__prompt_kernel(A_x, A_mem0, A_Wq, A_Wk, A_Wv, A_Wo, A_seg_len, B_x, B_w_gate, B_w_up, B_w_down, gate_w):
    B, S, DM = A_x.shape
    H, DH = A_Wq.shape[1], A_Wq.shape[2]
    M = A_mem0.shape[1]
    SEG = int(A_seg_len)
    DF = B_w_gate.shape[1]
    assert (B, S, DM, H, DH, M, SEG, DF) == (1, 2048, 640, 32, 128, 8, 32, 1728)
    L = M + SEG
    NP = S // (2 * SEG)
    HP = H // 2
    NT = DM // 128
    NU = 14
    DFP = NU * 128
    HU = NU // 2
    R0 = S // 2
    FM = 128
    scale = DH ** (-0.5)

    def kernel(x_hbm, mem0_ref, wq_hbm, wk_hbm, wv_hbm, wo_hbm, wgt_hbm, wut_hbm, wd_hbm, gw_ref,
               out_hbm,
               x_v, raw, wqkv, wo_v, wg_v, wu_v, wd_v, b_v, out_v, sems, osem):
        si = [0]

        def start(src, dst):
            cp = pltpu.make_async_copy(src, dst, sems.at[si[0]])
            si[0] += 1
            cp.start()
            return cp

        c_x0 = start(x_hbm.at[pl.ds(0, R0)], x_v.at[pl.ds(0, R0)])
        c_wg = start(wgt_hbm.bitcast(U32), wg_v.at[pl.ds(0, DF // 2)])
        c_wu = start(wut_hbm.bitcast(U32), wu_v.at[pl.ds(0, DF // 2)])
        c_wd = start(wd_hbm.bitcast(U32), wd_v.at[pl.ds(0, DF // 2)])
        c_qkv = []
        for wi, w_hbm in enumerate((wq_hbm, wk_hbm, wv_hbm)):
            w32 = w_hbm.bitcast(U32)
            for j in range(HP):
                for par in range(2):
                    c_qkv.append(start(w32.at[:, par, j, :], raw.at[wi, par, j]))
        c_wo = start(wo_hbm.bitcast(U32), wo_v)
        c_x1 = start(x_hbm.at[pl.ds(R0, S - R0)], x_v.at[pl.ds(R0, S - R0)])

        zpad = jnp.zeros(((DFP - DF) // 2, DM), U32)
        wg_v[pl.ds(DF // 2, (DFP - DF) // 2), :] = zpad
        wu_v[pl.ds(DF // 2, (DFP - DF) // 2), :] = zpad
        wd_v[pl.ds(DF // 2, (DFP - DF) // 2), :] = zpad

        def gu(xr, r64):
            g = _dot_nt(xr, _bf(wg_v[pl.ds(r64, 64), :]))
            u = _dot_nt(xr, _bf(wu_v[pl.ds(r64, 64), :]))
            return (jax.nn.gelu(g, approximate=True) * u).astype(BF)

        def down(h, k0, n):
            return _dot(h, _bf(wd_v[pl.ds(k0, HU * 64), pl.ds(n * 128, 128)]))

        c_x0.wait(); c_wg.wait(); c_wu.wait(); c_wd.wait()

        def ffn_body(i, c):
            r0 = pl.multiple_of(i * FM, FM)
            xr = x_v[pl.ds(r0, FM), :]
            for half in range(2):
                h = jnp.concatenate([gu(xr, (half * HU + u) * 64) for u in range(HU)], axis=1)
                for n in range(NT):
                    b_v[half, pl.ds(r0, FM), pl.ds(n * 128, 128)] = down(h, half * HU * 64, n)
            return c
        lax.fori_loop(0, R0 // FM, ffn_body, 0)

        for cp in c_qkv:
            cp.wait()

        def unzip(t, c):
            wi = t // HP
            j = t % HP
            a = raw[wi, 0, j]
            b = raw[wi, 1, j]
            wqkv[wi * H + 2 * j] = (a & U32(0xFFFF)) | (b << 16)
            wqkv[wi * H + 2 * j + 1] = (a >> 16) | (b & U32(0xFFFF0000))
            return c
        lax.fori_loop(0, 3 * HP, unzip, 0)
        c_wo.wait(); c_x1.wait()

        fill_e = _make_fill([(0, 32, 8), (32, 8, 0)], L, M)
        fill_o = _make_fill([(8, 24, 16), (32, 8, 8)], L, M)
        gw = gw_ref[...].astype(F32)

        def W(i):
            return _bf(wqkv[i])

        def step(lhs, even, saved, tail):
            fill = fill_e if even else fill_o
            st = [dict() for _ in range(HP)]
            acc = [None]

            def A(t):
                r = []
                for base in (0, H, 2 * H):
                    ys = []
                    for hh in range(2):
                        y = _dot(lhs, W(base + 2 * t + hh))
                        if even:
                            saved[(t, base, hh)] = y[32:40]
                            ys += [y[:32], y[40:48]]
                        else:
                            ys += [y, saved[(t, base, hh)]]
                    r.append(_cat0(*ys).astype(BF))
                st[t]["q"], st[t]["k"], st[t]["v"] = r

            def Bs(t):
                s = _dot_nt(st[t]["q"], st[t]["k"])
                s = jnp.where(fill == 0.0, s * scale, fill)
                m = jnp.max(s, axis=-1, keepdims=True)
                e = jnp.exp(s - m)
                st[t]["linv"] = 1.0 / jnp.sum(e, axis=-1, keepdims=True)
                st[t]["e"] = e.astype(BF)

            def C(t):
                o = _dot(st[t]["e"], st[t]["v"]) * st[t]["linv"]
                cols = []
                for hh in range(2):
                    oh = o[hh * L:(hh + 1) * L]
                    if even:
                        saved[(t, "o", hh)] = oh[24:32]
                        cols.append(_cat0(oh[:24], oh[32:40]))
                    else:
                        cols.append(_cat0(oh, saved[(t, "o", hh)]))
                st[t]["ol"] = jnp.concatenate(cols, axis=1).astype(BF)

            def D(t):
                y = _dot(st[t]["ol"], _bf(wo_v[pl.ds(t * 128, 128), :]))
                acc[0] = y if acc[0] is None else acc[0] + y

            for t in range(HP):
                A(t)
                if t >= 1: Bs(t - 1)
                if t >= 2: C(t - 2)
                if t >= 3: D(t - 3)
            Bs(HP - 1); C(HP - 2); D(HP - 3)
            for f in tail[0]: f()
            C(HP - 1); D(HP - 2)
            for f in tail[1]: f()
            D(HP - 1)
            for f in tail[2]: f()
            return acc[0]

        def body(p, mem):
            r0 = pl.multiple_of(p * (2 * SEG), 2 * SEG)
            xc = x_v[pl.ds(r0, 2 * SEG), :]
            half = p % 2
            fr0 = pl.multiple_of(R0 + (p // 2) * 64, 64)
            k0 = pl.multiple_of(half * (HU * 64), 64)
            xf = x_v[pl.ds(fr0, 64), :]
            hs = [None] * HU

            def f_gu(u):
                def f():
                    hs[u] = gu(xf, pl.multiple_of(k0 + u * 64, 64))
                return f

            def f_dn(n):
                def f():
                    h = jnp.concatenate(hs, axis=1)
                    b_v[half, pl.ds(fr0, 64), pl.ds(n * 128, 128)] = down(h, k0, n)
                return f

            saved = {}
            lhs = _cat0(xc[:40], mem)
            a_e = step(lhs, True, saved, {0: [f_gu(0), f_gu(1)], 1: [f_gu(2)], 2: [f_gu(3), f_gu(4)]})
            mem = a_e[24:32].astype(BF)
            lhs = _cat0(mem, xc[40:])
            a_o = step(lhs, False, saved, {0: [f_gu(5), f_gu(6), f_dn(0)], 1: [f_dn(1), f_dn(2), f_dn(3)], 2: [f_dn(4)]})
            mem = a_o[:M].astype(BF)
            a = _cat0(a_e[:24], a_o[40:48], a_o[32:40], a_o[8:32])
            b = b_v[0, pl.ds(r0, 2 * SEG), :] + b_v[1, pl.ds(r0, 2 * SEG), :]
            g = jax.nn.sigmoid(jnp.sum(xc.astype(F32) * gw, axis=-1, keepdims=True))
            out_v[pl.ds(r0, 2 * SEG), :] = (g * a + (1.0 - g) * b).astype(out_v.dtype)
            pltpu.make_async_copy(out_v.at[pl.ds(r0, 2 * SEG)], out_hbm.at[pl.ds(r0, 2 * SEG)], osem).start()
            return mem

        lax.fori_loop(0, NP, body, mem0_ref[...])
        pltpu.make_async_copy(out_v, out_hbm, osem).wait()

    hbm_spec = pl.BlockSpec(memory_space=pltpu.HBM)
    vmem_spec = pl.BlockSpec(memory_space=pltpu.VMEM)
    n_sems = 6 + 3 * H
    out = pl.pallas_call(
        kernel,
        out_shape=jax.ShapeDtypeStruct((S, DM), A_x.dtype),
        in_specs=[hbm_spec, vmem_spec, hbm_spec, hbm_spec, hbm_spec, hbm_spec, hbm_spec, hbm_spec, hbm_spec, vmem_spec],
        out_specs=hbm_spec,
        scratch_shapes=[
            pltpu.VMEM((S, DM), BF),
            pltpu.VMEM((3, 2, HP, DM // 2, DH), U32),
            pltpu.VMEM((3 * H, DM // 2, DH), U32),
            pltpu.VMEM((H * DH // 2, DM), U32),
            pltpu.VMEM((DFP // 2, DM), U32),
            pltpu.VMEM((DFP // 2, DM), U32),
            pltpu.VMEM((DFP // 2, DM), U32),
            pltpu.VMEM((2, S, DM), F32),
            pltpu.VMEM((S, DM), BF),
            pltpu.SemaphoreType.DMA((n_sems,)),
            pltpu.SemaphoreType.DMA,
        ],
        compiler_params=pltpu.CompilerParams(vmem_limit_bytes=110 * 1024 * 1024),
    )(
        A_x.reshape(S, DM), A_mem0.reshape(M, DM),
        A_Wq.reshape(DM // 2, 2, H, DH), A_Wk.reshape(DM // 2, 2, H, DH), A_Wv.reshape(DM // 2, 2, H, DH),
        A_Wo.reshape(H * DH, DM), B_w_gate.T, B_w_up.T, B_w_down, gate_w.reshape(1, DM),
    )
    return out.reshape(B, S, DM)
```

```python
import jax
import jax.numpy as jnp
from jax import lax
import jax.experimental.pallas as pl
import jax.experimental.pallas.tpu as pltpu

BF = jnp.bfloat16
F32 = jnp.float32
U32 = jnp.uint32


def _dot(a, b):
    return jnp.dot(a, b, preferred_element_type=F32)


def _dot_nt(a, b):
    return lax.dot_general(a, b, (((1,), (1,)), ((), ())), preferred_element_type=F32)


def _bf(w32):
    return pltpu.bitcast(w32, BF)


def _cat0(*xs):
    return jnp.concatenate(xs, axis=0)


def _gelu(x):
    return jax.nn.gelu(x, approximate=True)


def _mo(v, m):
    return v if isinstance(v, int) else pl.multiple_of(v, m)


def _make_fill(order, L, M):
    r = lax.broadcasted_iota(jnp.int32, (2 * L, 2 * L), 0)
    c = lax.broadcasted_iota(jnp.int32, (2 * L, 2 * L), 1)
    rl = jnp.where(r >= L, r - L, r)
    cl = jnp.where(c >= L, c - L, c)
    same = ((r >= L) & (c >= L)) | ((r < L) & (c < L))

    def pos(l):
        p = l
        for (st, n, p0) in order:
            p = jnp.where((l >= st) & (l < st + n), l - st + p0, p)
        return p
    rp = pos(rl)
    cp = pos(cl)
    allowed = (rp < M) | (rp >= cp)
    fill = jnp.where(allowed, 0.0, -1e9).astype(F32)
    fill = jnp.where(same, fill, -3e38).astype(F32)
    return fill


@jax.jit
def pallas_gated_mix__memory_aug_recurrent_mem_tr__glu_gated_geglu__prompt_kernel(A_x, A_mem0, A_Wq, A_Wk, A_Wv, A_Wo, A_seg_len, B_x, B_w_gate, B_w_up, B_w_down, gate_w):
    B, S, DM = A_x.shape
    H, DH = A_Wq.shape[1], A_Wq.shape[2]
    M = A_mem0.shape[1]
    SEG = 32
    DF = B_w_gate.shape[1]
    assert (B, S, DM, H, DH, M, SEG, DF) == (1, 2048, 640, 32, 128, 8, 32, 1728)
    L = M + SEG
    PR = 2 * SEG
    BR = 2 * PR
    NP = S // BR
    TAILS = [[1, 1, 0, 1, 2], [1, 1, 0, 1, 2], [1, 1, 0, 1, 1], [1, 1, 0, 1, 0]]
    LAGS = (2, 3)
    HP = H // 2
    NT = DM // 128
    NU = DF // 128
    HU = (NU - 1) // 2
    R0 = S // 2
    RB = 128
    NRB = R0 // RB
    XB = 512
    NXB = S // XB
    NSL = 3 * HP
    NG = NU - 1
    GS = NSL // NG
    UC = 40
    scale = DH ** (-0.5)
    S_X = 0
    S_F = S_X + NXB
    S_G = S_F + 3 * (NU + 1)
    S_WO = S_G + NG
    S_M = S_WO + 1
    S_GW = S_M + 1
    N_SEMS = S_GW + 1

    def kernel(x_hbm, mem0_hbm, wq_hbm, wk_hbm, wv_hbm, wo_hbm, wgt_hbm, wut_hbm, wd_hbm, gw_hbm,
               out_hbm,
               x_v, raw, wqkv, wo_v, wg_v, wu_v, wd_v, b_v, g_v, a_v, out_v, mem0_ref, gw_ref, sems, osem):
        f_src = (wgt_hbm.bitcast(U32), wut_hbm.bitcast(U32), wd_hbm.bitcast(U32))
        f_dst = (wg_v, wu_v, wd_v)
        w_src = (wq_hbm.bitcast(U32), wk_hbm.bitcast(U32), wv_hbm.bitcast(U32))
        x32 = x_hbm.bitcast(U32)

        def x_copy(i):
            sl = pl.ds(_mo(i * (XB // 2), XB // 2), XB // 2)
            return pltpu.make_async_copy(x32.at[sl], x_v.at[sl], sems.at[S_X + i])

        def X(r, n):
            return _bf(x_v[pl.ds(_mo(r // 2, 8), n // 2), :])

        def f_copy(u, k, n=64):
            r = _mo(u * 64, 64)
            return pltpu.make_async_copy(f_src[k].at[pl.ds(r, n)], f_dst[k].at[pl.ds(r, n)],
                                         sems.at[S_F + 3 * u + k])

        def g_start(g):
            for s in range(g * GS, (g + 1) * GS):
                wi, j = s // HP, s % HP
                pltpu.make_async_copy(w_src[wi].at[:, j, :], raw.at[s, pl.ds(0, DM)], sems.at[S_G + g]).start()

        def g_wait(g):
            blk = raw.at[pl.ds(g * GS, GS), pl.ds(0, DM)]
            pltpu.make_async_copy(blk, blk, sems.at[S_G + g]).wait()

        c_wo = pltpu.make_async_copy(wo_hbm.bitcast(U32), wo_v, sems.at[S_WO])

        def issue(g0, g1):
            for g in range(g0, g1):
                for k in range(3):
                    f_copy(g + 1, k).start()
                g_start(g)

        c_gw = pltpu.make_async_copy(gw_hbm, gw_ref, sems.at[S_GW])
        c_m = pltpu.make_async_copy(mem0_hbm, mem0_ref, sems.at[S_M])
        x_copy(0).start()
        c_gw.start()
        c_m.start()
        for k in range(3):
            f_copy(NU, k, 32).start()
        for k in range(3):
            f_copy(0, k).start()
        for i in range(1, NXB):
            x_copy(i).start()
        issue(0, 8)

        a_v[...] = jnp.zeros(a_v.shape, F32)
        c_gw.wait()
        c_m.wait()
        gw5 = gw_ref[...].astype(F32)

        for k in range(3):
            f_copy(NU, k, 32).wait()
        for k in range(3):
            f_copy(0, k).wait()

        def ffn_first(i, c):
            x_copy(i).wait()
            rr = NU * 64
            prev = None
            for rb in range(XB // RB + 1):
                if rb < XB // RB:
                    r = _mo(i * XB + rb * RB, RB)
                    xr = X(r, RB)
                    xf32 = xr.astype(F32)
                    zz = xf32[:, :128] * gw5[0:1]
                    for kt in range(1, NT):
                        zz = zz + xf32[:, kt * 128:(kt + 1) * 128] * gw5[kt:kt + 1]
                    gate = jax.nn.sigmoid(jnp.sum(zz, axis=-1, keepdims=True))
                    gate = jnp.broadcast_to(gate, (RB, 128))
                    g_v[pl.ds(r, RB), :] = gate
                    og = 1.0 - gate
                    y = _dot_nt(xr, _bf(_cat0(wg_v[pl.ds(rr, 32), :], wu_v[pl.ds(rr, 32), :])))
                    h1 = (_gelu(y[:, :64]) * y[:, 64:] * og[:, :64]).astype(BF)
                    h0 = (_gelu(_dot_nt(xr, _bf(wg_v[pl.ds(0, 64), :])))
                          * _dot_nt(xr, _bf(wu_v[pl.ds(0, 64), :])) * og).astype(BF)
                if prev is not None:
                    pr_, p1, p0 = prev
                    b_v[pl.ds(pr_, RB), :] = (_dot(p1, _bf(wd_v[pl.ds(rr, 32), :]))
                                              + _dot(p0, _bf(wd_v[pl.ds(0, 64), :])))
                prev = (r, h1, h0)
            return c
        lax.fori_loop(0, NXB, ffn_first, 0)
        issue(8, NG)
        c_wo.start()

        def unzip(s):
            for c0 in range(0, DM // 2, UC):
                a = raw[s, pl.ds(2 * c0, UC, stride=2), :]
                b = raw[s, pl.ds(2 * c0 + 1, UC, stride=2), :]
                wqkv[2 * s, pl.ds(c0, UC), :] = (a & U32(0xFFFF)) | (b << 16)
                wqkv[2 * s + 1, pl.ds(c0, UC), :] = (a >> 16) | (b & U32(0xFFFF0000))

        def ffn_loop(g, hcar):
            u = g + 1
            for k in range(3):
                f_copy(u, k).wait()
            g_wait(g)
            r = _mo(u * 64, 64)
            rp = _mo(g * 64, 64)
            hprev = hcar
            for rb in range(NRB):
                xr = X(rb * RB, RB)
                h = (_gelu(_dot_nt(xr, _bf(wg_v[pl.ds(r, 64), :])))
                     * _dot_nt(xr, _bf(wu_v[pl.ds(r, 64), :]))
                     * (1.0 - g_v[pl.ds(rb * RB, RB), :])).astype(BF)
                if rb == 0:
                    b_v[pl.ds((NRB - 1) * RB, RB), :] += _dot(hprev, _bf(wd_v[pl.ds(rp, 64), :]))
                else:
                    b_v[pl.ds((rb - 1) * RB, RB), :] += _dot(hprev, _bf(wd_v[pl.ds(r, 64), :]))
                hprev = h
                if rb % (NRB // GS) == 0:
                    unzip(g * GS + rb // (NRB // GS))
            return hprev
        hlast = lax.fori_loop(0, NG, ffn_loop, jnp.zeros((RB, 128), BF))
        b_v[pl.ds((NRB - 1) * RB, RB), :] += _dot(hlast, _bf(wd_v[pl.ds(NG * 64, 64), :]))

        c_wo.wait()

        fill_e = _make_fill([(0, 32, 8), (32, 8, 0)], L, M)
        fill_o = _make_fill([(8, 24, 16), (32, 8, 8)], L, M)

        def W(wi, h):
            return _bf(wqkv[wi * H + h])

        def step(lhs, even, saved, tail, lagc, mid=None):
            fill = fill_e if even else fill_o
            st = [dict() for _ in range(HP)]
            acc = [None]

            def A(t):
                r = []
                for wi in range(3):
                    ys = []
                    for hh in range(2):
                        y = _dot(lhs, W(wi, 2 * t + hh))
                        if even:
                            saved[(t, wi, hh)] = y[32:40]
                            ys += [y[:32], y[40:48]]
                        else:
                            ys += [y, saved[(t, wi, hh)]]
                    r.append(_cat0(*ys).astype(BF))
                st[t]["q"], st[t]["k"], st[t]["v"] = r

            def Bs(t):
                s = _dot_nt(st[t]["q"], st[t]["k"])
                s = jnp.where(fill == 0.0, s * scale, fill)
                m = jnp.max(s, axis=-1, keepdims=True)
                e = jnp.exp(s - m)
                st[t]["linv"] = 1.0 / jnp.sum(e, axis=-1, keepdims=True)
                st[t]["e"] = e.astype(BF)

            def C(t):
                o = _dot(st[t]["e"], st[t]["v"]) * st[t]["linv"]
                cols = []
                for hh in range(2):
                    oh = o[hh * L:(hh + 1) * L]
                    if even:
                        saved[(t, "o", hh)] = oh[24:32]
                        cols.append(_cat0(oh[:24], oh[32:40]))
                    else:
                        cols.append(_cat0(oh, saved[(t, "o", hh)]))
                st[t]["ol"] = jnp.concatenate(cols, axis=1).astype(BF)

            def D(t):
                y = _dot(st[t]["ol"], _bf(wo_v[pl.ds(t * 128, 128), :]))
                acc[0] = y if acc[0] is None else acc[0] + y

            lagd = lagc + 1
            for t in range(HP):
                A(t)
                if t == 0 and mid is not None:
                    mid()
                if t >= 1: Bs(t - 1)
                if t >= lagc: C(t - lagc)
                if t >= lagd: D(t - lagd)
            Bs(HP - 1)
            for t in range(HP - lagc, HP - 2):
                C(t); D(t - 1)
            for f in tail[0]: f()
            C(HP - 2); D(HP - 3)
            for f in tail[1]: f()
            C(HP - 1)
            for f in tail[2]: f()
            D(HP - 2)
            for f in tail[3]: f()
            D(HP - 1)
            for f in tail[4]: f()
            return acc[0]

        def combine(rq):
            for i in range(BR // 64):
                g = g_v[pl.ds(rq + i * 64, 64), :]
                for n in range(NT):
                    cs = pl.ds(n * 128, 128)
                    out_v[pl.ds(rq + i * 64, 64), cs] = (
                        g * a_v[pl.ds(i * 64, 64), cs] + b_v[pl.ds(rq + i * 64, 64), cs]).astype(out_v.dtype)

        def out_copy(rq):
            return pltpu.make_async_copy(out_v.at[pl.ds(rq, BR)], out_hbm.at[pl.ds(rq, BR)], osem)

        def body(p, mem):
            r0 = _mo(p * BR, BR)
            rq = _mo(jnp.maximum(p - 1, 0) * BR, BR)
            half = p % 2
            fr0 = _mo(R0 + (p // 2) * BR, BR)
            k0 = _mo(64 + half * (HU * 64), 64)
            gs = [None] * HU
            hs = [None] * HU

            def f_g(u):
                def f():
                    gs[u] = (_gelu(_dot_nt(X(fr0, BR), _bf(wg_v[pl.ds(_mo(k0 + u * 64, 64), 64), :])))
                             * (1.0 - g_v[pl.ds(fr0, BR), :]))
                return f

            def f_u(u):
                def f():
                    hs[u] = (gs[u] * _dot_nt(X(fr0, BR), _bf(wu_v[pl.ds(_mo(k0 + u * 64, 64), 64), :]))).astype(BF)
                return f

            def f_dn(n):
                def f():
                    h = jnp.concatenate(hs, axis=1)
                    b_v[pl.ds(fr0, BR), pl.ds(n * 128, 128)] += _dot(
                        h, _bf(wd_v[pl.ds(k0, HU * 64), pl.ds(n * 128, 128)]))
                return f

            fl = []
            for u in range(HU):
                fl += [f_g(u), f_u(u)]
            fl += [f_dn(n) for n in range(NT)]
            pos = [0]

            def take(counts):
                out = []
                for c in counts:
                    out.append(fl[pos[0]:pos[0] + c])
                    pos[0] += c
                return out

            for i in range(BR // PR):
                xc = X(r0 + i * PR, PR)
                saved = {}
                lhs = _cat0(xc[:40], mem)
                a_e = step(lhs, True, saved, take(TAILS[2 * i]), LAGS[0],
                           mid=(lambda: combine(rq)) if i == 0 else None)
                mem = a_e[24:32].astype(BF)
                a_v[pl.ds(i * PR, 24), :] = a_e[:24]
                lhs = _cat0(mem, xc[40:])
                a_o = step(lhs, False, saved, take(TAILS[2 * i + 1]), LAGS[1])
                mem = a_o[:M].astype(BF)
                a_v[pl.ds(i * PR + 24, 40), :] = _cat0(a_o[40:48], a_o[32:40], a_o[8:32])
            assert pos[0] == len(fl), (pos[0], len(fl))

            @pl.when(p > 0)
            def _():
                out_copy(rq).start()
            return mem

        lax.fori_loop(0, NP, body, mem0_ref[...])
        combine(S - BR)
        out_copy(S - BR).start()
        pltpu.make_async_copy(out_v, out_hbm, osem).wait()

    hbm_spec = pl.BlockSpec(memory_space=pltpu.HBM)
    vmem_spec = pl.BlockSpec(memory_space=pltpu.VMEM)
    out = pl.pallas_call(
        kernel,
        out_shape=jax.ShapeDtypeStruct((S, DM), A_x.dtype),
        in_specs=[hbm_spec] * 10,
        out_specs=hbm_spec,
        scratch_shapes=[
            pltpu.VMEM((S // 2, DM), U32),
            pltpu.VMEM((NSL, DM + 8, DH), U32),
            pltpu.VMEM((3 * H, DM // 2, DH), U32),
            pltpu.VMEM((H * DH // 2, DM), U32),
            pltpu.VMEM((DF // 2, DM), U32),
            pltpu.VMEM((DF // 2, DM), U32),
            pltpu.VMEM((DF // 2, DM), U32),
            pltpu.VMEM((S, DM), F32),
            pltpu.VMEM((S, 128), F32),
            pltpu.VMEM((BR, DM), F32),
            pltpu.VMEM((S, DM), BF),
            pltpu.VMEM((M, DM), BF),
            pltpu.VMEM((NT, 128), BF),
            pltpu.SemaphoreType.DMA((N_SEMS,)),
            pltpu.SemaphoreType.DMA,
        ],
        compiler_params=pltpu.CompilerParams(vmem_limit_bytes=110 * 1024 * 1024),
    )(
        A_x.reshape(S, DM), A_mem0.reshape(M, DM),
        A_Wq, A_Wk, A_Wv,
        A_Wo.reshape(H * DH, DM), B_w_gate.T, B_w_up.T, B_w_down, gate_w.reshape(NT, 128),
    )
    return out.reshape(B, S, DM)
```

```python
import jax
import jax.numpy as jnp
from jax import lax
import jax.experimental.pallas as pl
import jax.experimental.pallas.tpu as pltpu

BF = jnp.bfloat16
F32 = jnp.float32
U32 = jnp.uint32


def _dot(a, b):
    return jnp.dot(a, b, preferred_element_type=F32)


def _dot_nt(a, b):
    return lax.dot_general(a, b, (((1,), (1,)), ((), ())), preferred_element_type=F32)


def _bf(w32):
    return pltpu.bitcast(w32, BF)


def _cat0(*xs):
    return jnp.concatenate(xs, axis=0)


def _gelu(x):
    return jax.nn.gelu(x, approximate=True)


def _mo(v, m):
    return v if isinstance(v, int) else pl.multiple_of(v, m)


def _make_fill(order, L, M):
    r = lax.broadcasted_iota(jnp.int32, (2 * L, 2 * L), 0)
    c = lax.broadcasted_iota(jnp.int32, (2 * L, 2 * L), 1)
    rl = jnp.where(r >= L, r - L, r)
    cl = jnp.where(c >= L, c - L, c)
    same = ((r >= L) & (c >= L)) | ((r < L) & (c < L))

    def pos(l):
        p = l
        for (st, n, p0) in order:
            p = jnp.where((l >= st) & (l < st + n), l - st + p0, p)
        return p
    rp = pos(rl)
    cp = pos(cl)
    allowed = (rp < M) | (rp >= cp)
    fill = jnp.where(allowed, 0.0, -1e9).astype(F32)
    fill = jnp.where(same, fill, -3e38).astype(F32)
    return fill


@jax.jit
def pallas_gated_mix__memory_aug_recurrent_mem_tr__glu_gated_geglu__prompt_kernel(A_x, A_mem0, A_Wq, A_Wk, A_Wv, A_Wo, A_seg_len, B_x, B_w_gate, B_w_up, B_w_down, gate_w):
    B, S, DM = A_x.shape
    H, DH = A_Wq.shape[1], A_Wq.shape[2]
    M = A_mem0.shape[1]
    SEG = 32
    DF = B_w_gate.shape[1]
    assert (B, S, DM, H, DH, M, SEG, DF) == (1, 2048, 640, 32, 128, 8, 32, 1728)
    L = M + SEG
    PR = 2 * SEG
    BR = 2 * PR
    NP = S // BR
    TAILS = [[1, 1, 0, 1, 2], [1, 1, 0, 1, 2], [1, 1, 0, 1, 1], [1, 1, 0, 1, 0]]
    LAGS = (2, 3)
    HP = H // 2
    NT = DM // 128
    NU = DF // 128
    HU = (NU - 1) // 2
    R0 = S // 2
    RB = 128
    NRB = R0 // RB
    XB = 512
    NXB = S // XB
    NSL = 3 * HP
    UPI = 2
    NG = (NU - 1) // UPI
    GS = NSL // NG
    UC = 40
    NC = (DM // 2) // UC
    scale = DH ** (-0.5)
    S_X = 0
    S_0 = S_X + NXB
    S_F = S_0 + 1
    S_G = S_F + NG
    S_WO = S_G + NG
    N_SEMS = S_WO + 1

    def kernel(x_hbm, mem0_hbm, wq_hbm, wk_hbm, wv_hbm, wo_hbm, wgt_hbm, wut_hbm, wd_hbm, gw_hbm,
               out_hbm,
               x_v, raw, wqkv, wo_v, wg_v, wu_v, wd_v, b_v, g_v, a_v, out_v, mem0_ref, gw_ref, z_v,
               sems, osem):
        f_src = (wgt_hbm.bitcast(U32), wut_hbm.bitcast(U32), wd_hbm.bitcast(U32))
        f_dst = (wg_v, wu_v, wd_v)
        w_src = (wq_hbm.bitcast(U32), wk_hbm.bitcast(U32), wv_hbm.bitcast(U32))
        x32 = x_hbm.bitcast(U32)

        def x_copy(i):
            sl = pl.ds(_mo(i * (XB // 2), XB // 2), XB // 2)
            return pltpu.make_async_copy(x32.at[sl], x_v.at[sl], sems.at[S_X + i])

        def X(r, n):
            return _bf(x_v[pl.ds(_mo(r // 2, 8), n // 2), :])

        def f_copy(u, k, n, si):
            r = _mo(u * 64, 64)
            return pltpu.make_async_copy(f_src[k].at[pl.ds(r, n)], f_dst[k].at[pl.ds(r, n)], sems.at[si])

        def g_start(g):
            for s in range(g * GS, (g + 1) * GS):
                wi, j = s // HP, s % HP
                pltpu.make_async_copy(w_src[wi].at[:, j, :], raw.at[s, pl.ds(0, DM)],
                                      sems.at[S_G + g]).start()

        def g_wait(g):
            blk = raw.at[pl.ds(g * GS, GS), pl.ds(0, DM)]
            pltpu.make_async_copy(blk, blk, sems.at[S_G + g]).wait()

        c_wo = pltpu.make_async_copy(wo_hbm.bitcast(U32), wo_v, sems.at[S_WO])
        c_gw = pltpu.make_async_copy(gw_hbm, gw_ref, sems.at[S_0])
        c_m = pltpu.make_async_copy(mem0_hbm, mem0_ref, sems.at[S_0])

        x_copy(0).start()
        c_gw.start()
        c_m.start()
        for k in range(3):
            f_copy(NU, k, 32, S_0).start()
        for k in range(3):
            f_copy(0, k, 64, S_0).start()
        for i in range(1, NXB):
            x_copy(i).start()
        for g in range(NG):
            for k in range(3):
                f_copy(g * UPI + 1, k, 64 * UPI, S_F + g).start()
            g_start(g)
        c_wo.start()

        a_v[...] = jnp.zeros(a_v.shape, F32)
        z_v[...] = jnp.zeros(z_v.shape, U32)
        c_gw.wait()
        c_m.wait()
        for k in range(3):
            f_copy(NU, k, 32, S_0).wait()
        for k in range(3):
            f_copy(0, k, 64, S_0).wait()
        gw5 = gw_ref[...].astype(F32)

        def ffn_first(i, c):
            x_copy(i).wait()
            rr = NU * 64
            prev = None
            for rb in range(XB // RB + 1):
                if rb < XB // RB:
                    r = _mo(i * XB + rb * RB, RB)
                    xr = X(r, RB)
                    xf32 = xr.astype(F32)
                    zz = xf32[:, :128] * gw5[0:1]
                    for kt in range(1, NT):
                        zz = zz + xf32[:, kt * 128:(kt + 1) * 128] * gw5[kt:kt + 1]
                    gate = jax.nn.sigmoid(jnp.sum(zz, axis=-1, keepdims=True))
                    gate = jnp.broadcast_to(gate, (RB, 128))
                    g_v[pl.ds(r, RB), :] = gate
                    og = 1.0 - gate
                    y = _dot_nt(xr, _bf(_cat0(wg_v[pl.ds(rr, 32), :], wu_v[pl.ds(rr, 32), :])))
                    h1 = (_gelu(y[:, :64]) * y[:, 64:] * og[:, :64]).astype(BF)
                    h0 = (_gelu(_dot_nt(xr, _bf(wg_v[pl.ds(0, 64), :])))
                          * _dot_nt(xr, _bf(wu_v[pl.ds(0, 64), :])) * og).astype(BF)
                if prev is not None:
                    pr_, p1, p0 = prev
                    b_v[pl.ds(pr_, RB), :] = (_dot(p1, _bf(wd_v[pl.ds(rr, 32), :]))
                                              + _dot(p0, _bf(wd_v[pl.ds(0, 64), :])))
                prev = (r, h1, h0)
            return c
        lax.fori_loop(0, NXB, ffn_first, 0)

        def unzip(s, c0, src):
            dep = pltpu.bitcast(src[:8, :128], U32) & z_v[...]
            dep = jnp.concatenate([dep] * (UC // 8), axis=0)
            a = raw[s, pl.ds(2 * c0, UC, stride=2), :] | dep
            b = raw[s, pl.ds(2 * c0 + 1, UC, stride=2), :] | dep
            wqkv[2 * s, pl.ds(c0, UC), :] = (a & U32(0xFFFF)) | (b << 16)
            wqkv[2 * s + 1, pl.ds(c0, UC), :] = (a >> 16) | (b & U32(0xFFFF0000))

        def ffn_loop(g, hcar):
            u0 = g * UPI + 1
            for k in range(3):
                f_copy(u0, k, 64 * UPI, S_F + g).wait()
            g_wait(g)
            hprev = hcar
            nz = [0]

            def uz(src):
                if nz[0] < GS * NC:
                    unzip(g * GS + nz[0] // NC, (nz[0] % NC) * UC, src)
                    nz[0] += 1

            for ui in range(UPI):
                r = _mo((u0 + ui) * 64, 64)
                rp = _mo((u0 + ui - 1) * 64, 64)
                for rb in range(NRB):
                    xr = X(rb * RB, RB)
                    gm = _dot_nt(xr, _bf(wg_v[pl.ds(r, 64), :]))
                    um = _dot_nt(xr, _bf(wu_v[pl.ds(r, 64), :]))
                    h = (_gelu(gm) * um * (1.0 - g_v[pl.ds(rb * RB, RB), :])).astype(BF)
                    if rb == 0:
                        dn = _dot(hprev, _bf(wd_v[pl.ds(rp, 64), :]))
                        b_v[pl.ds((NRB - 1) * RB, RB), :] += dn
                    else:
                        dn = _dot(hprev, _bf(wd_v[pl.ds(r, 64), :]))
                        b_v[pl.ds((rb - 1) * RB, RB), :] += dn
                    hprev = h
                    for src in (gm, um, dn, dn[:, 512:], gm[64:]):
                        uz(src)
            assert nz[0] == GS * NC
            return hprev
        hlast = lax.fori_loop(0, NG, ffn_loop, jnp.zeros((RB, 128), BF))
        b_v[pl.ds((NRB - 1) * RB, RB), :] += _dot(hlast, _bf(wd_v[pl.ds((NU - 1) * 64, 64), :]))

        fill_e = _make_fill([(0, 32, 8), (32, 8, 0)], L, M)
        fill_o = _make_fill([(8, 24, 16), (32, 8, 8)], L, M)
        c_wo.wait()

        def step(lhs, even, saved, tail, lagc, mid=None):
            fill = fill_e if even else fill_o
            st = [dict() for _ in range(HP)]
            acc = [None]

            def A(t):
                r = []
                for wi in range(3):
                    ys = []
                    for hh in range(2):
                        y = _dot(lhs, _bf(wqkv[wi * H + 2 * t + hh]))
                        if even:
                            saved[(t, wi, hh)] = y[32:40]
                            ys += [y[:32], y[40:48]]
                        else:
                            ys += [y, saved[(t, wi, hh)]]
                    r.append(_cat0(*ys).astype(BF))
                st[t]["q"], st[t]["k"], st[t]["v"] = r

            def Bs(t):
                s = _dot_nt(st[t]["q"], st[t]["k"])
                s = jnp.where(fill == 0.0, s * scale, fill)
                m = jnp.max(s, axis=-1, keepdims=True)
                e = jnp.exp(s - m)
                st[t]["linv"] = 1.0 / jnp.sum(e, axis=-1, keepdims=True)
                st[t]["e"] = e.astype(BF)

            def C(t):
                o = _dot(st[t]["e"], st[t]["v"]) * st[t]["linv"]
                cols = []
                for hh in range(2):
                    oh = o[hh * L:(hh + 1) * L]
                    if even:
                        saved[(t, "o", hh)] = oh[24:32]
                        cols.append(_cat0(oh[:24], oh[32:40]))
                    else:
                        cols.append(_cat0(oh, saved[(t, "o", hh)]))
                st[t]["ol"] = jnp.concatenate(cols, axis=1).astype(BF)

            def D(t):
                y = _dot(st[t]["ol"], _bf(wo_v[pl.ds(t * 128, 128), :]))
                acc[0] = y if acc[0] is None else acc[0] + y

            lagd = lagc + 1
            for t in range(HP):
                A(t)
                if t == 0 and mid is not None:
                    mid()
                if t >= 1:
                    Bs(t - 1)
                if t >= lagc:
                    C(t - lagc)
                if t >= lagd:
                    D(t - lagd)
            Bs(HP - 1)
            for t in range(HP - lagc, HP - 2):
                C(t)
                D(t - 1)
            for f in tail[0]:
                f()
            C(HP - 2)
            D(HP - 3)
            for f in tail[1]:
                f()
            C(HP - 1)
            for f in tail[2]:
                f()
            D(HP - 2)
            for f in tail[3]:
                f()
            D(HP - 1)
            for f in tail[4]:
                f()
            return acc[0]

        def out_copy(rq, n=BR):
            return pltpu.make_async_copy(out_v.at[pl.ds(rq, n)], out_hbm.at[pl.ds(rq, n)], osem)

        def combine(rq, last=False):
            for i in range(BR // 64):
                g = g_v[pl.ds(rq + i * 64, 64), :]
                for n in range(NT):
                    cs = pl.ds(n * 128, 128)
                    out_v[pl.ds(rq + i * 64, 64), cs] = (
                        g * a_v[pl.ds(i * 64, 64), cs] + b_v[pl.ds(rq + i * 64, 64), cs]).astype(out_v.dtype)
                if last:
                    out_copy(rq + i * 64, 64).start()

        def body(p, mem):
            r0 = _mo(p * BR, BR)
            rq = _mo(jnp.maximum(p - 1, 0) * BR, BR)
            fr0 = _mo(R0 + (p // 2) * BR, BR)
            k0 = _mo(64 + (p % 2) * (HU * 64), 64)
            gs = [None] * HU
            hs = [None] * HU

            def f_g(u):
                def f():
                    gs[u] = (_gelu(_dot_nt(X(fr0, BR), _bf(wg_v[pl.ds(_mo(k0 + u * 64, 64), 64), :])))
                             * (1.0 - g_v[pl.ds(fr0, BR), :]))
                return f

            def f_u(u):
                def f():
                    hs[u] = (gs[u] * _dot_nt(X(fr0, BR),
                                             _bf(wu_v[pl.ds(_mo(k0 + u * 64, 64), 64), :]))).astype(BF)
                return f

            def f_dn(n):
                def f():
                    h = jnp.concatenate(hs, axis=1)
                    b_v[pl.ds(fr0, BR), pl.ds(n * 128, 128)] += _dot(
                        h, _bf(wd_v[pl.ds(k0, HU * 64), pl.ds(n * 128, 128)]))
                return f

            fl = []
            for u in range(HU):
                fl += [f_g(u), f_u(u)]
            fl += [f_dn(n) for n in range(NT)]
            pos = [0]

            def take(counts):
                out = []
                for c in counts:
                    out.append(fl[pos[0]:pos[0] + c])
                    pos[0] += c
                return out

            for i in range(BR // PR):
                xc = X(r0 + i * PR, PR)
                saved = {}
                a_e = step(_cat0(xc[:40], mem), True, saved, take(TAILS[2 * i]), LAGS[0],
                           mid=(lambda: combine(rq)) if i == 0 else None)
                mem = a_e[24:32].astype(BF)
                a_v[pl.ds(i * PR, 24), :] = a_e[:24]
                a_o = step(_cat0(mem, xc[40:]), False, saved, take(TAILS[2 * i + 1]), LAGS[1])
                mem = a_o[:M].astype(BF)
                a_v[pl.ds(i * PR + 24, 40), :] = _cat0(a_o[40:48], a_o[32:40], a_o[8:32])
            assert pos[0] == len(fl), (pos[0], len(fl))

            @pl.when(p > 0)
            def _():
                out_copy(rq).start()
            return mem

        lax.fori_loop(0, NP, body, mem0_ref[...])
        combine(S - BR, last=True)
        pltpu.make_async_copy(out_v, out_hbm, osem).wait()

    hbm_spec = pl.BlockSpec(memory_space=pltpu.HBM)
    out = pl.pallas_call(
        kernel,
        out_shape=jax.ShapeDtypeStruct((S, DM), A_x.dtype),
        in_specs=[hbm_spec] * 10,
        out_specs=hbm_spec,
        scratch_shapes=[
            pltpu.VMEM((S // 2, DM), U32),
            pltpu.VMEM((NSL, DM + 8, DH), U32),
            pltpu.VMEM((3 * H, DM // 2, DH), U32),
            pltpu.VMEM((H * DH // 2, DM), U32),
            pltpu.VMEM((DF // 2, DM), U32),
            pltpu.VMEM((DF // 2, DM), U32),
            pltpu.VMEM((DF // 2, DM), U32),
            pltpu.VMEM((S, DM), F32),
            pltpu.VMEM((S, 128), F32),
            pltpu.VMEM((BR, DM), F32),
            pltpu.VMEM((S, DM), BF),
            pltpu.VMEM((M, DM), BF),
            pltpu.VMEM((NT, 128), BF),
            pltpu.VMEM((8, 128), U32),
            pltpu.SemaphoreType.DMA((N_SEMS,)),
            pltpu.SemaphoreType.DMA,
        ],
        compiler_params=pltpu.CompilerParams(vmem_limit_bytes=110 * 1024 * 1024),
    )(
        A_x.reshape(S, DM), A_mem0.reshape(M, DM),
        A_Wq, A_Wk, A_Wv,
        A_Wo.reshape(H * DH, DM), B_w_gate.T, B_w_up.T, B_w_down, gate_w.reshape(NT, 128),
    )
    return out.reshape(B, S, DM)
```

```python
import jax
import jax.numpy as jnp
from jax import lax
import jax.experimental.pallas as pl
import jax.experimental.pallas.tpu as pltpu

BF = jnp.bfloat16
F32 = jnp.float32
U32 = jnp.uint32


def _dot(a, b):
    return jnp.dot(a, b, preferred_element_type=F32)


def _dot_nt(a, b):
    return lax.dot_general(a, b, (((1,), (1,)), ((), ())), preferred_element_type=F32)


def _bf(w32):
    return pltpu.bitcast(w32, BF)


def _cat0(*xs):
    return jnp.concatenate(xs, axis=0)


def _gelu(x):
    return jax.nn.gelu(x, approximate=True)


def _mo(v, m):
    return v if isinstance(v, int) else pl.multiple_of(v, m)


def _make_fill(order, L, M):
    r = lax.broadcasted_iota(jnp.int32, (2 * L, 2 * L), 0)
    c = lax.broadcasted_iota(jnp.int32, (2 * L, 2 * L), 1)
    rl = jnp.where(r >= L, r - L, r)
    cl = jnp.where(c >= L, c - L, c)
    same = ((r >= L) & (c >= L)) | ((r < L) & (c < L))

    def pos(l):
        p = l
        for (st, n, p0) in order:
            p = jnp.where((l >= st) & (l < st + n), l - st + p0, p)
        return p
    rp = pos(rl)
    cp = pos(cl)
    allowed = (rp < M) | (rp >= cp)
    fill = jnp.where(allowed, 0.0, -1e9).astype(F32)
    fill = jnp.where(same, fill, -3e38).astype(F32)
    return fill


@jax.jit
def pallas_gated_mix__memory_aug_recurrent_mem_tr__glu_gated_geglu__prompt_kernel(A_x, A_mem0, A_Wq, A_Wk, A_Wv, A_Wo, A_seg_len, B_x, B_w_gate, B_w_up, B_w_down, gate_w):
    B, S, DM = A_x.shape
    H, DH = A_Wq.shape[1], A_Wq.shape[2]
    M = A_mem0.shape[1]
    SEG = 32
    DF = B_w_gate.shape[1]
    assert (B, S, DM, H, DH, M, SEG, DF) == (1, 2048, 640, 32, 128, 8, 32, 1728)
    L = M + SEG
    PR = 2 * SEG
    BR = 2 * PR
    NP = S // BR
    TAILS = [[1, 1, 0, 1, 2], [1, 1, 0, 1, 2], [1, 1, 0, 1, 1], [1, 1, 0, 1, 0]]
    LAGS = (2, 3)
    HP = H // 2
    NT = DM // 128
    NU = DF // 128
    HU = (NU - 1) // 2
    R0 = S // 2
    RB = 128
    NRB = R0 // RB
    XB = 512
    NXB = S // XB
    NSL = 3 * HP
    UPI = 2
    NG = (NU - 1) // UPI
    GS = NSL // NG
    UC = 40
    NC = (DM // 2) // UC
    scale = DH ** (-0.5)
    S_X = 0
    S_0 = S_X + NXB
    S_F = S_0 + 1
    S_G = S_F + NG
    S_WO = S_G + NG
    N_SEMS = S_WO + 1

    def kernel(x_hbm, mem0_hbm, wq_hbm, wk_hbm, wv_hbm, wo_hbm, wgt_hbm, wut_hbm, wd_hbm, gw_hbm,
               out_hbm,
               x_v, raw, wqkv, wo_v, wg_v, wu_v, wd_v, b_v, g_v, a_v, out_v, mem0_ref, gw_ref, z_v,
               sems, osem):
        f_src = (wgt_hbm.bitcast(U32), wut_hbm.bitcast(U32), wd_hbm.bitcast(U32))
        f_dst = (wg_v, wu_v, wd_v)
        w_src = (wq_hbm.bitcast(U32), wk_hbm.bitcast(U32), wv_hbm.bitcast(U32))
        x32 = x_hbm.bitcast(U32)

        def x_copy(i):
            sl = pl.ds(_mo(i * (XB // 2), XB // 2), XB // 2)
            return pltpu.make_async_copy(x32.at[sl], x_v.at[sl], sems.at[S_X + i])

        def X(r, n):
            return _bf(x_v[pl.ds(_mo(r // 2, 8), n // 2), :])

        def f_copy(u, k, n, si):
            r = _mo(u * 64, 64)
            return pltpu.make_async_copy(f_src[k].at[pl.ds(r, n)], f_dst[k].at[pl.ds(r, n)], sems.at[si])

        def g_start(g):
            for s in range(g * GS, (g + 1) * GS):
                wi, j = s // HP, s % HP
                pltpu.make_async_copy(w_src[wi].at[:, j, :], raw.at[s, pl.ds(0, DM)],
                                      sems.at[S_G + g]).start()

        def g_wait(g):
            blk = raw.at[pl.ds(g * GS, GS), pl.ds(0, DM)]
            pltpu.make_async_copy(blk, blk, sems.at[S_G + g]).wait()

        c_wo = pltpu.make_async_copy(wo_hbm.bitcast(U32), wo_v, sems.at[S_WO])
        c_gw = pltpu.make_async_copy(gw_hbm, gw_ref, sems.at[S_0])
        c_m = pltpu.make_async_copy(mem0_hbm, mem0_ref, sems.at[S_0])

        x_copy(0).start()
        c_gw.start()
        c_m.start()
        for k in range(3):
            f_copy(NU, k, 32, S_0).start()
        for k in range(3):
            f_copy(0, k, 64, S_0).start()
        for i in range(1, NXB):
            x_copy(i).start()
        for g in range(NG):
            for k in range(3):
                f_copy(g * UPI + 1, k, 64 * UPI, S_F + g).start()
            g_start(g)
        c_wo.start()

        a_v[...] = jnp.zeros(a_v.shape, F32)
        z_v[...] = jnp.zeros(z_v.shape, U32)
        c_gw.wait()
        c_m.wait()
        for k in range(3):
            f_copy(NU, k, 32, S_0).wait()
        for k in range(3):
            f_copy(0, k, 64, S_0).wait()
        gw5 = gw_ref[...].astype(F32)

        def ffn_first(i, c):
            x_copy(i).wait()
            rr = NU * 64
            prev = None
            for rb in range(XB // RB + 1):
                if rb < XB // RB:
                    r = _mo(i * XB + rb * RB, RB)
                    xr = X(r, RB)
                    xf32 = xr.astype(F32)
                    zz = xf32[:, :128] * gw5[0:1]
                    for kt in range(1, NT):
                        zz = zz + xf32[:, kt * 128:(kt + 1) * 128] * gw5[kt:kt + 1]
                    gate = jax.nn.sigmoid(jnp.sum(zz, axis=-1, keepdims=True))
                    gate = jnp.broadcast_to(gate, (RB, 128))
                    g_v[pl.ds(r, RB), :] = gate
                    og = 1.0 - gate
                    y = _dot_nt(xr, _bf(_cat0(wg_v[pl.ds(rr, 32), :], wu_v[pl.ds(rr, 32), :])))
                    h1 = (_gelu(y[:, :64]) * y[:, 64:] * og[:, :64]).astype(BF)
                    h0 = (_gelu(_dot_nt(xr, _bf(wg_v[pl.ds(0, 64), :])))
                          * _dot_nt(xr, _bf(wu_v[pl.ds(0, 64), :])) * og).astype(BF)
                if prev is not None:
                    pr_, p1, p0 = prev
                    b_v[pl.ds(pr_, RB), :] = (_dot(p1, _bf(wd_v[pl.ds(rr, 32), :]))
                                              + _dot(p0, _bf(wd_v[pl.ds(0, 64), :])))
                prev = (r, h1, h0)
            return c
        lax.fori_loop(0, NXB, ffn_first, 0)

        def unzip(s, c0, src):
            dep = pltpu.bitcast(src[:8, :128], U32) & z_v[...]
            dep = jnp.concatenate([dep] * (UC // 8), axis=0)
            a = raw[s, pl.ds(2 * c0, UC, stride=2), :] | dep
            b = raw[s, pl.ds(2 * c0 + 1, UC, stride=2), :] | dep
            wqkv[2 * s, pl.ds(c0, UC), :] = (a & U32(0xFFFF)) | (b << 16)
            wqkv[2 * s + 1, pl.ds(c0, UC), :] = (a >> 16) | (b & U32(0xFFFF0000))

        def ffn_loop(g, hcar):
            u0 = g * UPI + 1
            for k in range(3):
                f_copy(u0, k, 64 * UPI, S_F + g).wait()
            g_wait(g)
            hprev = hcar
            nz = [0]

            def uz(src):
                if nz[0] < GS * NC:
                    unzip(g * GS + nz[0] // NC, (nz[0] % NC) * UC, src)
                    nz[0] += 1

            for ui in range(UPI):
                r = _mo((u0 + ui) * 64, 64)
                rp = _mo((u0 + ui - 1) * 64, 64)
                for rb in range(NRB):
                    def down_prev():
                        d = _dot(hprev, _bf(wd_v[pl.ds(rp if rb == 0 else r, 64), :]))
                        b_v[pl.ds(((rb - 1) % NRB) * RB, RB), :] += d
                        return d

                    first = rb == 0 and ui == 0
                    if first:
                        dn = down_prev()
                    xr = X(rb * RB, RB)
                    gm = _dot_nt(xr, _bf(wg_v[pl.ds(r, 64), :]))
                    um = _dot_nt(xr, _bf(wu_v[pl.ds(r, 64), :]))
                    h = (_gelu(gm) * um * (1.0 - g_v[pl.ds(rb * RB, RB), :])).astype(BF)
                    if not first:
                        dn = down_prev()
                    hprev = h
                    for src in (gm, um, dn, dn[:, 512:], gm[64:]):
                        uz(src)
            assert nz[0] == GS * NC
            return hprev
        hlast = lax.fori_loop(0, NG, ffn_loop, jnp.zeros((RB, 128), BF))
        b_v[pl.ds((NRB - 1) * RB, RB), :] += _dot(hlast, _bf(wd_v[pl.ds((NU - 1) * 64, 64), :]))

        fill_e = _make_fill([(0, 32, 8), (32, 8, 0)], L, M)
        fill_o = _make_fill([(8, 24, 16), (32, 8, 8)], L, M)
        c_wo.wait()

        def step(lhs, even, saved, tail, lagc, mid=None):
            fill = fill_e if even else fill_o
            st = [dict() for _ in range(HP)]
            acc = [None]

            def A(t):
                r = []
                for wi in range(3):
                    ys = []
                    for hh in range(2):
                        y = _dot(lhs, _bf(wqkv[wi * H + 2 * t + hh]))
                        if even:
                            saved[(t, wi, hh)] = y[32:40]
                            ys += [y[:32], y[40:48]]
                        else:
                            ys += [y, saved[(t, wi, hh)]]
                    r.append(_cat0(*ys).astype(BF))
                st[t]["q"], st[t]["k"], st[t]["v"] = r

            def Bs(t):
                s = _dot_nt(st[t]["q"], st[t]["k"])
                s = jnp.where(fill == 0.0, s * scale, fill)
                m = jnp.max(s, axis=-1, keepdims=True)
                e = jnp.exp(s - m)
                st[t]["linv"] = 1.0 / jnp.sum(e, axis=-1, keepdims=True)
                st[t]["e"] = e.astype(BF)

            def C(t):
                o = _dot(st[t]["e"], st[t]["v"]) * st[t]["linv"]
                cols = []
                for hh in range(2):
                    oh = o[hh * L:(hh + 1) * L]
                    if even:
                        saved[(t, "o", hh)] = oh[24:32]
                        cols.append(_cat0(oh[:24], oh[32:40]))
                    else:
                        cols.append(_cat0(oh, saved[(t, "o", hh)]))
                st[t]["ol"] = jnp.concatenate(cols, axis=1).astype(BF)

            def D(t):
                y = _dot(st[t]["ol"], _bf(wo_v[pl.ds(t * 128, 128), :]))
                acc[0] = y if acc[0] is None else acc[0] + y

            lagd = lagc + 1
            for t in range(HP):
                A(t)
                if t == 0 and mid is not None:
                    mid()
                if t >= 1:
                    Bs(t - 1)
                if t >= lagc:
                    C(t - lagc)
                if t >= lagd:
                    D(t - lagd)
            Bs(HP - 1)
            for t in range(HP - lagc, HP - 2):
                C(t)
                D(t - 1)
            for f in tail[0]:
                f()
            C(HP - 2)
            D(HP - 3)
            for f in tail[1]:
                f()
            C(HP - 1)
            for f in tail[2]:
                f()
            D(HP - 2)
            for f in tail[3]:
                f()
            D(HP - 1)
            for f in tail[4]:
                f()
            return acc[0]

        def out_copy(rq, n=BR):
            return pltpu.make_async_copy(out_v.at[pl.ds(rq, n)], out_hbm.at[pl.ds(rq, n)], osem)

        def combine(rq, last=False):
            for i in range(BR // 64):
                g = g_v[pl.ds(rq + i * 64, 64), :]
                for n in range(NT):
                    cs = pl.ds(n * 128, 128)
                    out_v[pl.ds(rq + i * 64, 64), cs] = (
                        g * a_v[pl.ds(i * 64, 64), cs] + b_v[pl.ds(rq + i * 64, 64), cs]).astype(out_v.dtype)
                if last:
                    out_copy(rq + i * 64, 64).start()

        def body(p, mem):
            r0 = _mo(p * BR, BR)
            rq = _mo(jnp.maximum(p - 1, 0) * BR, BR)
            fr0 = _mo(R0 + (p // 2) * BR, BR)
            k0 = _mo(64 + (p % 2) * (HU * 64), 64)
            gs = [None] * HU
            hs = [None] * HU

            def f_g(u):
                def f():
                    gs[u] = (_gelu(_dot_nt(X(fr0, BR), _bf(wg_v[pl.ds(_mo(k0 + u * 64, 64), 64), :])))
                             * (1.0 - g_v[pl.ds(fr0, BR), :]))
                return f

            def f_u(u):
                def f():
                    hs[u] = (gs[u] * _dot_nt(X(fr0, BR),
                                             _bf(wu_v[pl.ds(_mo(k0 + u * 64, 64), 64), :]))).astype(BF)
                return f

            def f_dn(n):
                def f():
                    h = jnp.concatenate(hs, axis=1)
                    b_v[pl.ds(fr0, BR), pl.ds(n * 128, 128)] += _dot(
                        h, _bf(wd_v[pl.ds(k0, HU * 64), pl.ds(n * 128, 128)]))
                return f

            fl = []
            for u in range(HU):
                fl += [f_g(u), f_u(u)]
            fl += [f_dn(n) for n in range(NT)]
            pos = [0]

            def take(counts):
                out = []
                for c in counts:
                    out.append(fl[pos[0]:pos[0] + c])
                    pos[0] += c
                return out

            for i in range(BR // PR):
                xc = X(r0 + i * PR, PR)
                saved = {}
                a_e = step(_cat0(xc[:40], mem), True, saved, take(TAILS[2 * i]), LAGS[0],
                           mid=(lambda: combine(rq)) if i == 0 else None)
                mem = a_e[24:32].astype(BF)
                a_v[pl.ds(i * PR, 24), :] = a_e[:24]
                a_o = step(_cat0(mem, xc[40:]), False, saved, take(TAILS[2 * i + 1]), LAGS[1])
                mem = a_o[:M].astype(BF)
                a_v[pl.ds(i * PR + 24, 40), :] = _cat0(a_o[40:48], a_o[32:40], a_o[8:32])
            assert pos[0] == len(fl), (pos[0], len(fl))

            @pl.when(p > 0)
            def _():
                out_copy(rq).start()
            return mem

        lax.fori_loop(0, NP, body, mem0_ref[...])
        combine(S - BR, last=True)
        pltpu.make_async_copy(out_v, out_hbm, osem).wait()

    hbm_spec = pl.BlockSpec(memory_space=pltpu.HBM)
    out = pl.pallas_call(
        kernel,
        out_shape=jax.ShapeDtypeStruct((S, DM), A_x.dtype),
        in_specs=[hbm_spec] * 10,
        out_specs=hbm_spec,
        scratch_shapes=[
            pltpu.VMEM((S // 2, DM), U32),
            pltpu.VMEM((NSL, DM + 8, DH), U32),
            pltpu.VMEM((3 * H, DM // 2, DH), U32),
            pltpu.VMEM((H * DH // 2, DM), U32),
            pltpu.VMEM((DF // 2, DM), U32),
            pltpu.VMEM((DF // 2, DM), U32),
            pltpu.VMEM((DF // 2, DM), U32),
            pltpu.VMEM((S, DM), F32),
            pltpu.VMEM((S, 128), F32),
            pltpu.VMEM((BR, DM), F32),
            pltpu.VMEM((S, DM), BF),
            pltpu.VMEM((M, DM), BF),
            pltpu.VMEM((NT, 128), BF),
            pltpu.VMEM((8, 128), U32),
            pltpu.SemaphoreType.DMA((N_SEMS,)),
            pltpu.SemaphoreType.DMA,
        ],
        compiler_params=pltpu.CompilerParams(vmem_limit_bytes=110 * 1024 * 1024),
    )(
        A_x.reshape(S, DM), A_mem0.reshape(M, DM),
        A_Wq, A_Wk, A_Wv,
        A_Wo.reshape(H * DH, DM), B_w_gate.T, B_w_up.T, B_w_down, gate_w.reshape(NT, 128),
    )
    return out.reshape(B, S, DM)
```
